```python
import jax
import jax.numpy as jnp

def _softmax(x, axis=-1):
    return jax.nn.softmax(x, axis=axis)
def _gelu(x):
    return jax.nn.gelu(x, approximate=True)
def _silu(x):
    return jax.nn.silu(x)
def _sigmoid(x):
    return jax.nn.sigmoid(x)
def _layernorm(x, axis=-1, eps=1e-5):
    m = jnp.mean(x, axis=axis, keepdims=True)
    v = jnp.var(x, axis=axis, keepdims=True)
    return (x - m) / jnp.sqrt(v + eps)
def _scatter_add(tgt, idx, src, axis=0):
    return tgt.at[idx].add(src)
def _segment_sum(src, seg, n):
    return jax.ops.segment_sum(src, seg, n)
class _Rng:
    def __init__(self, key):
        self._k = key
    def _next(self):
        self._k, sub = jax.random.split(self._k)
        return sub
    def normal(self, shape):
        return jax.random.normal(self._next(), shape, dtype=jnp.bfloat16)
    def randint(self, lo, hi, shape):
        return jax.random.randint(self._next(), shape, lo, hi, dtype=jnp.int32)
    def uniform(self, shape, lo=0.0, hi=1.0):
        return jax.random.uniform(self._next(), shape, jnp.bfloat16, lo, hi)
    def permutation(self, n):
        return jax.random.permutation(self._next(), n)


kernel_name = 'recurrent_scan__sliding_local_dilated__glu_gated_swiglu__prompt'

def setup_inputs():
    _rng = _Rng(jax.random.key(int.from_bytes(__import__("os").urandom(4), "little")))
    _w = (lambda a: (lambda t: t.astype(jnp.bfloat16) if jnp.issubdtype(t.dtype, jnp.floating) else t)(jnp.asarray(a)))
    def _A_setup():
        B, S, D = 1, 2048, 1024
        return {
            "x": _w((lambda *s: _rng.normal(s) * 0.05)(B, S, D)),
            "wqkv": _w((lambda *s: _rng.normal(s) * 0.05)(D, 3 * D)),
            "wo": _w((lambda *s: _rng.normal(s) * 0.05)(D, D)),
        }
    _A_in = _A_setup()

    def _B_setup():
        B, S, D, F = 1, 2048, 1024, 3584
        return {
            "x": _w((lambda *s: _rng.normal(s) * 0.05)(B, S, D)),
            "w1": _w((lambda *s: _rng.normal(s) * 0.05)(D, F) * (2.0 / D) ** 0.5),
            "w3": _w((lambda *s: _rng.normal(s) * 0.05)(D, F) * (2.0 / D) ** 0.5),
            "w2": _w((lambda *s: _rng.normal(s) * 0.05)(F, D) * (2.0 / F) ** 0.5),
        }
    _B_in = _B_setup()

    return {
        "A_x": _A_in["x"],
        "A_wqkv": _A_in["wqkv"],
        "A_wo": _A_in["wo"],
        "B_x": _B_in["x"],
        "B_w1": _B_in["w1"],
        "B_w3": _B_in["w3"],
        "B_w2": _B_in["w2"],
    }

def reference(A_x, A_wqkv, A_wo, B_x, B_w1, B_w3, B_w2):
    def _A_ref(x, wqkv, wo):
        B, S, D = x.shape
        H = 32; Dh = D // H
        W, dil = 8, 2
        qkv = (lambda x, *d: x.transpose(*d))((x @ wqkv).reshape(B, S, 3, H, Dh), 2, 0, 3, 1, 4)
        q, k, v = qkv[0], qkv[1], qkv[2]
        scale = Dh ** -0.5
        pos = jnp.arange(S)
        off = jnp.arange(W) * dil
        idx = pos[:, None] - off[None, :]
        mask = idx >= 0
        idx_c = jnp.where(mask, idx, 0).reshape(-1)
        kg = k[:, :, idx_c, :].reshape(B, H, S, W, Dh)
        vg = v[:, :, idx_c, :].reshape(B, H, S, W, Dh)
        logits = jnp.einsum("bhsd,bhswd->bhsw", q, kg) * scale
        logits = jnp.where(mask[None, None, :, :], logits, -1e9)
        attn = _softmax(logits, axis=-1)
        o = jnp.einsum("bhsw,bhswd->bhsd", attn, vg)
        return (lambda x, *d: x.transpose(*d))(o, 0, 2, 1, 3).reshape(B, S, D) @ wo

    def _B_ref(x, w1, w3, w2):
        gate = jnp.einsum("bsd,df->bsf", x, w1)
        up = jnp.einsum("bsd,df->bsf", x, w3)
        h = _silu(gate) * up
        out = jnp.einsum("bsf,fd->bsd", h, w2)
        return out

    x = A_x
    xn = _layernorm(x, axis=-1)
    s = _A_ref(xn, A_wqkv, A_wo)
    g = _silu(_B_ref(xn, B_w1, B_w3, B_w2))
    return x + s * g
```

```python
import functools
import numpy as np
import jax
import jax.numpy as jnp
from jax import lax
from jax.experimental import pallas as pl
from jax.experimental.pallas import tpu as pltpu

F32 = jnp.float32
BF16 = jnp.bfloat16
U32 = jnp.uint32
S, D, F = 2048, 1024, 3584
H, DH, W, DIL = 32, 32, 8, 2
LOG2E = 1.4426950408889634
HALO = 16


def _dot(a, b):
    return jnp.dot(a, b, preferred_element_type=F32)


def _perm3(tiles, masks):
    for b in range(3):
        r = 4 << b
        m = masks[b]
        new = list(tiles)
        for c in range(8):
            if c & (1 << b):
                continue
            A, B = tiles[c], tiles[c | (1 << b)]
            new[c] = jnp.where(m, A, pltpu.roll(B, r, 1))
            new[c | (1 << b)] = jnp.where(m, pltpu.roll(A, 128 - r, 1), B)
        tiles = new
    return tiles


import contextlib
def make_kernel(scopes=False, flags=None, T=256, T0=512, FC=512, R=32, attn_slots=(1, 2, 3, 4), wo_slot=6, prep_slot=0, packed_perm=True):
    nT = S // T
    sc = (lambda n: jax.named_scope(n)) if scopes else (lambda n: contextlib.nullcontext())
    nF = F // FC
    nM = S // T0
    nR = T // R

    def kernel(x_hbm, wqkv_hbm, wo_hbm, w1_hbm, w3_hbm, w2_hbm, o_hbm,
               x_v, wqkv_v, wo_v, w1_v, w3_v, w2_v, xn_v, qkv_v, q_scr, k_scr, v_scr, o_scr, out_v,
               xsem, wsem, osem):

        def x_copy(m):
            return pltpu.make_async_copy(x_hbm.at[pl.ds(m * T0, T0), :], x_v.at[pl.ds(m * T0, T0), :], xsem.at[m])

        def qkv_copy(p):
            return pltpu.make_async_copy(wqkv_hbm.at[:, pl.ds(p * D, D)], wqkv_v.at[p], wsem.at[p])

        HF = F // 2

        def out_copy(t, slot):
            return pltpu.make_async_copy(out_v.at[slot], o_hbm.at[pl.ds(t * T, T), :], osem.at[slot])

        def w1_copy(c):
            return pltpu.make_async_copy(w1_hbm.at[:, pl.ds(c * HF, HF)], w1_v.at[:, pl.ds(c * HF, HF)], wsem.at[4 + c])
        def w3_copy(c):
            return pltpu.make_async_copy(w3_hbm.at[:, pl.ds(c * HF, HF)], w3_v.at[:, pl.ds(c * HF, HF)], wsem.at[6 + c])
        def w2_copy(c):
            return pltpu.make_async_copy(w2_hbm.at[pl.ds(c * HF, HF), :], w2_v.at[pl.ds(c * HF, HF), :], wsem.at[8 + c])
        wo_copy = pltpu.make_async_copy(wo_hbm, wo_v, wsem.at[3])
        x_copy(0).start()
        qkv_copy(0).start()
        x_copy(1).start()
        late0 = [[x_copy(2), qkv_copy(1)], [x_copy(3), qkv_copy(2)], [wo_copy], [w1_copy(0)]]
        late1 = [[w1_copy(1)], [w3_copy(0)], [w3_copy(1)], [w2_copy(0)], [w2_copy(1)], [], [], []]

        z = jnp.zeros((HALO, 128), F32)
        for e in range(8):
            k_scr[e, pl.ds(0, HALO), :] = z
            v_scr[e, pl.ds(0, HALO), :] = z

        def layernorm(r0):
            x = x_v[pl.ds(r0, T0), :].astype(F32)
            mu = jnp.mean(x, axis=-1, keepdims=True)
            xc = x - mu
            var = jnp.mean(xc * xc, axis=-1, keepdims=True)
            xn_v[pl.ds(r0, T0), :] = (xc / jnp.sqrt(var + 1e-5)).astype(BF16)

        with sc('a_wait_x0'):
            x_copy(0).wait()
        with sc('b_ln0'):
            layernorm(0)
        with sc('c_wait_wq'):
            qkv_copy(0).wait()

        def q_body(m, _):
            r0 = pl.multiple_of(m * T0, T0)

            for i, cs in enumerate(late0):
                @pl.when(m == i)
                def _(cs=cs):
                    for c in cs:
                        c.start()

            @pl.when(m + 1 < nM)
            def _():
                x_copy(m + 1).wait()
            qkv_v[0, pl.ds(r0, T0), :] = _dot(xn_v[pl.ds(r0, T0), :], wqkv_v[0]).astype(BF16)
            layernorm(pl.multiple_of(jnp.minimum(m + 1, nM - 1) * T0, T0))
            return 0
        with sc('d_L0'):
            lax.fori_loop(0, nM, q_body, 0)

        def kv_body(i, _):
            p = 1 + i // nM
            m = i % nM
            r0 = pl.multiple_of(m * T0, T0)

            for k, cs in enumerate(late1):
                if cs:
                    @pl.when(i == k)
                    def _(cs=cs):
                        for c in cs:
                            c.start()

            @pl.when(m == 0)
            def _():
                qkv_copy(p).wait()
            qkv_v[p, pl.ds(r0, T0), :] = _dot(xn_v[pl.ds(r0, T0), :], wqkv_v[p]).astype(BF16)
            return 0
        with sc('e_L1'):
            lax.fori_loop(0, 2 * nM, kv_body, 0)

        with sc('f_wait_w'):
            for c in [wo_copy, w1_copy(0), w1_copy(1), w3_copy(0), w3_copy(1), w2_copy(0), w2_copy(1)]:
                c.wait()

        laneR = lax.broadcasted_iota(jnp.int32, (R, 128), 1)
        m1 = (laneR & 1) == 0
        m2 = (laneR & 2) == 0
        laneH = lax.broadcasted_iota(jnp.int32, (R // 2, 128), 1)
        masksH = [(laneH & (4 << b)) == 0 for b in range(3)]
        rowR = lax.broadcasted_iota(jnp.int32, (R, 128), 0)
        laneP = lax.broadcasted_iota(jnp.int32, (T // 2, 128), 1)
        masksP = [(laneP & (4 << b)) == 0 for b in range(3)]

        def tile_body(t, _):
            t0 = pl.multiple_of(t * T, T)
            slot = t % 2

            @pl.when(t >= 2)
            def _():
                out_copy(t - 2, slot).wait()

            def prep():
                for part, (dst, off) in enumerate(((q_scr, 0), (k_scr, HALO), (v_scr, HALO))):
                    raw = pltpu.bitcast(qkv_v[part, pl.ds(t0, T), :], U32)
                    tiles = [raw[:, c * 128:(c + 1) * 128] for c in range(8)]
                    tiles = _perm3(tiles, masksP)
                    for e in range(8):
                        dst[e, pl.ds(off, T), :] = pltpu.bitcast(tiles[e], BF16).astype(F32)

            def attn_block(rb):
                r0 = rb * R
                q = [q_scr[e, pl.ds(r0, R), :] for e in range(8)]
                ls = []
                for j in range(W):
                    a = None
                    for e in range(8):
                        p = q[e] * k_scr[e, pl.ds(HALO + r0 - DIL * j, R), :]
                        a = p if a is None else a + p
                    a = a + jnp.where(m1, pltpu.roll(a, 127, 1), pltpu.roll(a, 1, 1))
                    a = a + jnp.where(m2, pltpu.roll(a, 126, 1), pltpu.roll(a, 2, 1))
                    a = a * DH ** -0.5
                    if r0 < DIL * j:
                        a = jnp.where(t0 + r0 + rowR >= DIL * j, a, -1e9)
                    ls.append(a)
                m = ls[0]
                for j in range(1, W):
                    m = jnp.maximum(m, ls[j])
                ps = [jnp.exp(l - m) for l in ls]
                z = ps[0]
                for j in range(1, W):
                    z = z + ps[j]
                inv = 1.0 / z
                outs = []
                for e in range(8):
                    a = None
                    for j in range(W):
                        p = ps[j] * v_scr[e, pl.ds(HALO + r0 - DIL * j, R), :]
                        a = p if a is None else a + p
                    outs.append(pltpu.bitcast((a * inv).astype(BF16), U32))
                outs = _perm3(outs, masksH)
                for c in range(8):
                    o_scr[pl.ds(r0, R), pl.ds(c * 128, 128)] = pltpu.bitcast(outs[c], BF16)

            per = -(-nR // len(attn_slots))
            sched = {s: list(range(i * per, min(nR, (i + 1) * per))) for i, s in enumerate(attn_slots)}

            xn = xn_v[pl.ds(t0, T), :]
            acc = None
            s_out = None
            for c in range(nF):
                g = _dot(xn, w1_v[:, pl.ds(c * FC, FC)])
                u = _dot(xn, w3_v[:, pl.ds(c * FC, FC)])
                if c == prep_slot:
                    prep()
                for rb in sched.get(c, []):
                    attn_block(rb)
                h = (g * jax.nn.sigmoid(g) * u).astype(BF16)
                p = _dot(h, w2_v[pl.ds(c * FC, FC), :])
                acc = p if acc is None else acc + p
                if c == wo_slot:
                    s_out = _dot(o_scr[...], wo_v[...])

            for e in range(8):
                k_scr[e, pl.ds(0, HALO), :] = k_scr[e, pl.ds(T, HALO), :]
                v_scr[e, pl.ds(0, HALO), :] = v_scr[e, pl.ds(T, HALO), :]

            gate = acc * jax.nn.sigmoid(acc)
            out_v[slot] = (x_v[pl.ds(t0, T), :].astype(F32) + s_out * gate).astype(BF16)
            out_copy(t, slot).start()
            return 0

        with sc('g_main'):
            lax.fori_loop(0, nT, tile_body, 0)
        with sc('h_tail'):
            out_copy(nT - 2, (nT - 2) % 2).wait()
            out_copy(nT - 1, (nT - 1) % 2).wait()

    def fn(A_x, A_wqkv, A_wo, B_x, B_w1, B_w3, B_w2):
        del B_x
        x = A_x.reshape(S, D)
        any_ = pl.BlockSpec(memory_space=pl.ANY)
        out = pl.pallas_call(
            kernel,
            in_specs=[any_] * 6,
            out_specs=any_,
            out_shape=jax.ShapeDtypeStruct((S, D), A_x.dtype),
            scratch_shapes=[
                pltpu.VMEM((S, D), BF16),
                pltpu.VMEM((3, D, D), BF16), pltpu.VMEM((D, D), BF16),
                pltpu.VMEM((D, F), BF16), pltpu.VMEM((D, F), BF16), pltpu.VMEM((F, D), BF16),
                pltpu.VMEM((S, D), BF16), pltpu.VMEM((3, S, D), BF16),
                pltpu.VMEM((8, T, 128), F32), pltpu.VMEM((8, HALO + T, 128), F32), pltpu.VMEM((8, HALO + T, 128), F32),
                pltpu.VMEM((T, D), BF16), pltpu.VMEM((2, T, D), BF16),
                pltpu.SemaphoreType.DMA((nM,)), pltpu.SemaphoreType.DMA((10,)), pltpu.SemaphoreType.DMA((2,)),
            ],
            compiler_params=pltpu.CompilerParams(vmem_limit_bytes=110 * 1024 * 1024, flags=flags),
        )(x, A_wqkv, A_wo, B_w1, B_w3, B_w2)
        return out.reshape(1, S, D)
    return fn


_impl = make_kernel(flags={'XLA_TPU_EVENLY_DISTRIBUTE_CRITICAL_NODES': True})


@jax.jit
def pallas_recurrent_scan__sliding_local_dilated__glu_gated_swiglu__prompt_kernel(
    A_x: jax.Array,
    A_wqkv: jax.Array,
    A_wo: jax.Array,
    B_x: jax.Array,
    B_w1: jax.Array,
    B_w3: jax.Array,
    B_w2: jax.Array,
):
    return _impl(A_x, A_wqkv, A_wo, B_x, B_w1, B_w3, B_w2)
```

```python
import functools
import numpy as np
import jax
import jax.numpy as jnp
from jax import lax
from jax.experimental import pallas as pl
from jax.experimental.pallas import tpu as pltpu

F32 = jnp.float32
BF16 = jnp.bfloat16
U32 = jnp.uint32
S, D, F = 2048, 1024, 3584
H, DH, W, DIL = 32, 32, 8, 2
LOG2E = 1.4426950408889634
HALO = 16


def _dot(a, b):
    return jnp.dot(a, b, preferred_element_type=F32)


def _perm3(tiles, masks):
    for b in range(3):
        r = 4 << b
        m = masks[b]
        new = list(tiles)
        for c in range(8):
            if c & (1 << b):
                continue
            A, B = tiles[c], tiles[c | (1 << b)]
            new[c] = jnp.where(m, A, pltpu.roll(B, r, 1))
            new[c | (1 << b)] = jnp.where(m, pltpu.roll(A, 128 - r, 1), B)
        tiles = new
    return tiles


import contextlib
def make_kernel(scopes=False, flags=None, silu='tanh', nq=4, xsplit=True, osplit=1, starts=((2, (0, 1)), (3, (2,)), (4, (3,)), (5, (4,)), (6, (5,)), (7, (6,))), kvwait=4, T=256, T0=512, FC=512, R=32, attn_slots=(1, 2, 3, 4), wo_slot=6, prep_slot=0, packed_perm=True):
    nT = S // T

    def silu_mul(g, u):
        if silu == 'tanh':
            hg = 0.5 * g
            return (hg + hg * jnp.tanh(hg)) * u
        return g * jax.nn.sigmoid(g) * u
    sc = (lambda n: jax.named_scope(n)) if scopes else (lambda n: contextlib.nullcontext())
    nF = F // FC
    nM = S // T0
    nR = T // R

    def kernel(x_hbm, wqkv_hbm, wo_hbm, w1_hbm, w3_hbm, w2_hbm, o_hbm,
               x_v, wqkv_v, wo_v, w1_v, w3_v, w2_v, xn_v, qkv_v, q_scr, k_scr, v_scr, o_scr, out_v,
               xsem, wsem, osem, qsem):

        HF = F // 2
        QN = D // nq

        def x_copy(m):
            return pltpu.make_async_copy(x_hbm.at[pl.ds(m * T0, T0), :], x_v.at[pl.ds(m * T0, T0), :], xsem.at[m])

        def q_copy(n):
            return pltpu.make_async_copy(wqkv_hbm.at[:, pl.ds(n * QN, QN)], wqkv_v.at[0, :, pl.ds(n * QN, QN)], qsem.at[n])

        def kv_copy(p):
            return pltpu.make_async_copy(wqkv_hbm.at[:, pl.ds(p * D, D)], wqkv_v.at[p], wsem.at[p])

        def out_copy(t, slot):
            return pltpu.make_async_copy(out_v.at[slot], o_hbm.at[pl.ds(t * T, T), :], osem.at[slot])

        def w1_copy(c):
            return pltpu.make_async_copy(w1_hbm.at[:, pl.ds(c * HF, HF)], w1_v.at[:, pl.ds(c * HF, HF)], wsem.at[4 + c])

        def w3_copy(c):
            return pltpu.make_async_copy(w3_hbm.at[:, pl.ds(c * HF, HF)], w3_v.at[:, pl.ds(c * HF, HF)], wsem.at[6 + c])

        def w2_copy(c):
            return pltpu.make_async_copy(w2_hbm.at[pl.ds(c * HF, HF), :], w2_v.at[pl.ds(c * HF, HF), :], wsem.at[8 + c])
        wo_copy = pltpu.make_async_copy(wo_hbm, wo_v, wsem.at[3])

        def layernorm(src0, dst0):
            x = x_v[pl.ds(src0, T0), :].astype(F32)
            mu = jnp.mean(x, axis=-1, keepdims=True)
            xc = x - mu
            var = jnp.mean(xc * xc, axis=-1, keepdims=True)
            xn_v[pl.ds(dst0, T0), :] = (xc / jnp.sqrt(var + 1e-5)).astype(BF16)

        HT = T0 // 2
        xa_copy = pltpu.make_async_copy(x_hbm.at[pl.ds(0, HT), :], x_v.at[pl.ds(0, HT), :], xsem.at[0])
        xb_copy = pltpu.make_async_copy(x_hbm.at[pl.ds(HT, HT), :], x_v.at[pl.ds(HT, HT), :], xsem.at[nM])
        big = [wo_copy, w1_copy(0), w1_copy(1), w3_copy(0), w3_copy(1), w2_copy(0), w2_copy(1)]
        if xsplit:
            xa_copy.start()
            q_copy(0).start()
            xb_copy.start()
        else:
            x_copy(0).start()
            for n in range(nq):
                q_copy(n).start()
            x_copy(1).start()

        z = jnp.zeros((HALO, 128), F32)
        for e in range(8):
            k_scr[e, pl.ds(0, HALO), :] = z
            v_scr[e, pl.ds(0, HALO), :] = z

        def ln_rows(r0, n):
            x = x_v[pl.ds(r0, n), :].astype(F32)
            mu = jnp.mean(x, axis=-1, keepdims=True)
            xc = x - mu
            var = jnp.mean(xc * xc, axis=-1, keepdims=True)
            xn_v[pl.ds(r0, n), :] = (xc / jnp.sqrt(var + 1e-5)).astype(BF16)

        def q_dot(r0, n, c0):
            qkv_v[0, pl.ds(r0, n), pl.ds(c0, QN)] = _dot(xn_v[pl.ds(r0, n), :], wqkv_v[0, :, pl.ds(c0, QN)]).astype(BF16)

        def mid_starts():
            x_copy(1).wait()
            for c in (x_copy(2), x_copy(3)):
                c.start()

        if xsplit:
            with sc('a_wait_x0'):
                xa_copy.wait()
            with sc('b_ln0'):
                ln_rows(0, HT)
            with sc('c_q0'):
                q_copy(1).start()
                q_copy(0).wait()
                q_dot(0, HT, 0)
                xb_copy.wait()
                for n in range(2, nq):
                    q_copy(n).start()
                x_copy(1).start()
                ln_rows(HT, HT)
                q_dot(HT, HT, 0)
                for n in range(1, nq):
                    q_copy(n).wait()
                    if n == nq - 1:
                        mid_starts()
                    q_dot(0, T0, n * QN)
                layernorm(T0, T0)
        else:
            with sc('a_wait_x0'):
                x_copy(0).wait()
            with sc('b_ln0'):
                layernorm(0, 0)
            with sc('c_q0'):
                for n in range(nq):
                    q_copy(n).wait()
                    if n == nq - 1:
                        mid_starts()
                    q_dot(0, T0, n * QN)
                layernorm(T0, T0)

        def proj_body(i, _):
            p = i // nM
            m = i % nM
            r0 = pl.multiple_of(m * T0, T0)
            acts = {1: [x_copy(2).wait, kv_copy(1).start, kv_copy(2).start], 2: [x_copy(3).wait]}
            acts.setdefault(kvwait, []).extend([kv_copy(1).wait, kv_copy(2).wait])
            for k, idx in starts:
                acts.setdefault(k, []).extend([big[j].start for j in idx])
            for k, fs in sorted(acts.items()):
                @pl.when(i == k)
                def _(fs=fs):
                    for f in fs:
                        f()
            qkv_v[p, pl.ds(r0, T0), :] = _dot(xn_v[pl.ds(r0, T0), :], wqkv_v[p]).astype(BF16)
            layernorm(pl.multiple_of(jnp.minimum(i + 1, nM - 1) * T0, T0), pl.multiple_of(jnp.minimum(i + 1, nM) * T0, T0))
            return 0
        with sc('d_L0'):
            lax.fori_loop(1, 3 * nM, proj_body, 0)

        with sc('f_wait_w'):
            for c in big:
                c.wait()

        laneR = lax.broadcasted_iota(jnp.int32, (R, 128), 1)
        m1 = (laneR & 1) == 0
        m2 = (laneR & 2) == 0
        laneH = lax.broadcasted_iota(jnp.int32, (R // 2, 128), 1)
        masksH = [(laneH & (4 << b)) == 0 for b in range(3)]
        rowR = lax.broadcasted_iota(jnp.int32, (R, 128), 0)
        laneP = lax.broadcasted_iota(jnp.int32, (T // 2, 128), 1)
        masksP = [(laneP & (4 << b)) == 0 for b in range(3)]

        def tile_body(t, _):
            t0 = pl.multiple_of(t * T, T)
            slot = t % 2

            @pl.when(t >= 2)
            def _():
                out_copy(t - 2, slot).wait()

            def prep():
                for part, (dst, off) in enumerate(((q_scr, 0), (k_scr, HALO), (v_scr, HALO))):
                    raw = pltpu.bitcast(qkv_v[part, pl.ds(t0, T), :], U32)
                    tiles = [raw[:, c * 128:(c + 1) * 128] for c in range(8)]
                    tiles = _perm3(tiles, masksP)
                    for e in range(8):
                        dst[e, pl.ds(off, T), :] = pltpu.bitcast(tiles[e], BF16).astype(F32)

            def attn_block(rb):
                r0 = rb * R
                q = [q_scr[e, pl.ds(r0, R), :] for e in range(8)]
                ls = []
                for j in range(W):
                    a = None
                    for e in range(8):
                        p = q[e] * k_scr[e, pl.ds(HALO + r0 - DIL * j, R), :]
                        a = p if a is None else a + p
                    a = a + jnp.where(m1, pltpu.roll(a, 127, 1), pltpu.roll(a, 1, 1))
                    a = a + jnp.where(m2, pltpu.roll(a, 126, 1), pltpu.roll(a, 2, 1))
                    if r0 < DIL * j:
                        a = jnp.where(t0 + r0 + rowR >= DIL * j, a, -1e9 / DH ** -0.5)
                    ls.append(a)
                m = ls[0]
                for j in range(1, W):
                    m = jnp.maximum(m, ls[j])
                ps = [jnp.exp2((l - m) * (LOG2E * DH ** -0.5)) for l in ls]
                z = ps[0]
                for j in range(1, W):
                    z = z + ps[j]
                inv = 1.0 / z
                outs = []
                for e in range(8):
                    a = None
                    for j in range(W):
                        p = ps[j] * v_scr[e, pl.ds(HALO + r0 - DIL * j, R), :]
                        a = p if a is None else a + p
                    outs.append(pltpu.bitcast((a * inv).astype(BF16), U32))
                outs = _perm3(outs, masksH)
                for c in range(8):
                    o_scr[pl.ds(r0, R), pl.ds(c * 128, 128)] = pltpu.bitcast(outs[c], BF16)

            sched = {}
            for rb in range(nR):
                sched.setdefault(attn_slots[rb * len(attn_slots) // nR], []).append(rb)

            xn = xn_v[pl.ds(t0, T), :]
            acc = None
            s_out = None
            for c in range(nF):
                g = _dot(xn, w1_v[:, pl.ds(c * FC, FC)])
                u = _dot(xn, w3_v[:, pl.ds(c * FC, FC)])
                if c == prep_slot:
                    prep()
                for rb in sched.get(c, []):
                    attn_block(rb)
                h = silu_mul(g, u).astype(BF16)
                p = _dot(h, w2_v[pl.ds(c * FC, FC), :])
                acc = p if acc is None else acc + p
                if c == wo_slot:
                    s_out = _dot(o_scr[...], wo_v[...])

            for e in range(8):
                k_scr[e, pl.ds(0, HALO), :] = k_scr[e, pl.ds(T, HALO), :]
                v_scr[e, pl.ds(0, HALO), :] = v_scr[e, pl.ds(T, HALO), :]

            out_v[slot] = (x_v[pl.ds(t0, T), :].astype(F32) + silu_mul(acc, s_out)).astype(BF16)
            out_copy(t, slot).start()
            return 0

        with sc('g_main'):
            lax.fori_loop(0, nT, tile_body, 0)
        with sc('h_tail'):
            out_copy(nT - 2, (nT - 2) % 2).wait()
            out_copy(nT - 1, (nT - 1) % 2).wait()

    def fn(A_x, A_wqkv, A_wo, B_x, B_w1, B_w3, B_w2):
        del B_x
        x = A_x.reshape(S, D)
        any_ = pl.BlockSpec(memory_space=pl.ANY)
        out = pl.pallas_call(
            kernel,
            in_specs=[any_] * 6,
            out_specs=any_,
            out_shape=jax.ShapeDtypeStruct((S, D), A_x.dtype),
            scratch_shapes=[
                pltpu.VMEM((S, D), BF16),
                pltpu.VMEM((3, D, D), BF16), pltpu.VMEM((D, D), BF16),
                pltpu.VMEM((D, F), BF16), pltpu.VMEM((D, F), BF16), pltpu.VMEM((F, D), BF16),
                pltpu.VMEM((S + T0, D), BF16), pltpu.VMEM((3, S, D), BF16),
                pltpu.VMEM((8, T, 128), F32), pltpu.VMEM((8, HALO + T, 128), F32), pltpu.VMEM((8, HALO + T, 128), F32),
                pltpu.VMEM((T, D), BF16), pltpu.VMEM((2, T, D), BF16),
                pltpu.SemaphoreType.DMA((nM + 1,)), pltpu.SemaphoreType.DMA((10,)), pltpu.SemaphoreType.DMA((2,)), pltpu.SemaphoreType.DMA((nq,)),
            ],
            compiler_params=pltpu.CompilerParams(vmem_limit_bytes=110 * 1024 * 1024, flags=flags),
        )(x, A_wqkv, A_wo, B_w1, B_w3, B_w2)
        return out.reshape(1, S, D)
    return fn


_impl = make_kernel(flags={'XLA_TPU_EVENLY_DISTRIBUTE_CRITICAL_NODES': True}, nq=2)


@jax.jit
def pallas_recurrent_scan__sliding_local_dilated__glu_gated_swiglu__prompt_kernel(
    A_x: jax.Array,
    A_wqkv: jax.Array,
    A_wo: jax.Array,
    B_x: jax.Array,
    B_w1: jax.Array,
    B_w3: jax.Array,
    B_w2: jax.Array,
):
    return _impl(A_x, A_wqkv, A_wo, B_x, B_w1, B_w3, B_w2)
```

```python
import contextlib

import jax
import jax.numpy as jnp
from jax import lax
from jax.experimental import pallas as pl
from jax.experimental.pallas import tpu as pltpu

F32 = jnp.float32
BF16 = jnp.bfloat16
U32 = jnp.uint32
S, D, F = 2048, 1024, 3584
H, DH, W, DIL = 32, 32, 8, 2
LOG2E = 1.4426950408889634
HALO = 16
HK, HF = D // 2, F // 2


def _dot(a, b):
    return jnp.dot(a, b, preferred_element_type=F32)


def _perm3(tiles, masks):
    for b in range(3):
        r = 4 << b
        m = masks[b]
        new = list(tiles)
        for c in range(8):
            if c & (1 << b):
                continue
            A, B = tiles[c], tiles[c | (1 << b)]
            new[c] = jnp.where(m, A, pltpu.roll(B, r, 1))
            new[c | (1 << b)] = jnp.where(m, pltpu.roll(A, 128 - r, 1), B)
        tiles = new
    return tiles


def _silu_mul(g, u):
    hg = 0.5 * g
    return (hg + hg * jnp.tanh(hg)) * u


def _left_operands(a11, a12, a21, a22):
    return [a11 + a22, a21 + a22, a11, a22, a11 + a12, a21 - a11, a12 - a22]


def _right_sums(b11, b12, b21, b22):
    return [b11 + b22, b12 - b22, b21 - b11, b11 + b12, b21 + b22]


def _products(L, sums, b11, b22):
    R = [sums[0], b11, sums[1], sums[2], b22, sums[3], sums[4]]
    return [_dot(l, r) for l, r in zip(L, R)]


def _combine(M):
    return (M[0] + M[3] - M[4] + M[6], M[2] + M[4], M[1] + M[3], M[0] - M[1] + M[2] + M[5])


def make_kernel(scopes=False, flags=None, T=256, T0=512, NC=256, R=32, nsub=16, sqparts=16, xsplit=False):
    nT, nM, nC, nR = S // T, S // T0, HF // NC, T // R
    sc = (lambda n: jax.named_scope(n)) if scopes else (lambda n: contextlib.nullcontext())

    def kernel(x_hbm, wqkv_hbm, wo_hbm, w1_hbm, w3_hbm, w2_hbm, o_hbm,
               x_v, wqkv_v, wo_v, w1_v, w3_v, w2_v, r1_v, r3_v, r2_v, rq_v, xn_v, qkv_v,
               q_scr, k_scr, v_scr, o_scr, out_v, xsem, wsem, osem):

        HT = T0 // 2

        def x_rows(r0, n, k):
            return pltpu.make_async_copy(x_hbm.at[pl.ds(r0, n), :], x_v.at[pl.ds(r0, n), :], xsem.at[k])

        def x_copy(m):
            return x_rows(m * T0, T0, m)

        def qkv_copy(p):
            return pltpu.make_async_copy(wqkv_hbm.at[:, pl.ds(p * D, D)], wqkv_v.at[p], wsem.at[p])

        def cols_copy(src, dst, c, k):
            return pltpu.make_async_copy(src.at[:, pl.ds(c * HF, HF)], dst.at[:, pl.ds(c * HF, HF)], wsem.at[k])

        def rows_copy(src, dst, c, k):
            return pltpu.make_async_copy(src.at[pl.ds(c * HF, HF), :], dst.at[pl.ds(c * HF, HF), :], wsem.at[k])

        late = [cols_copy(w1_hbm, w1_v, 0, 3), cols_copy(w1_hbm, w1_v, 1, 4),
                cols_copy(w3_hbm, w3_v, 0, 5), cols_copy(w3_hbm, w3_v, 1, 6),
                rows_copy(w2_hbm, w2_v, 0, 7), rows_copy(w2_hbm, w2_v, 1, 8),
                pltpu.make_async_copy(wo_hbm, wo_v, wsem.at[9])]

        def out_copy(t, slot):
            return pltpu.make_async_copy(out_v.at[slot], o_hbm.at[pl.ds(t * T, T), :], osem.at[slot])

        def when_step(i, acts):
            for k, fs in sorted(acts.items()):
                @pl.when(i == k)
                def _(fs=fs):
                    for f in fs:
                        f()

        def ln_rows(src0, dst0, n):
            x = x_v[pl.ds(src0, n), :].astype(F32)
            mu = jnp.mean(x, axis=-1, keepdims=True)
            xc = x - mu
            var = jnp.mean(xc * xc, axis=-1, keepdims=True)
            xn_v[pl.ds(dst0, n), :] = (xc / jnp.sqrt(var + 1e-5)).astype(BF16)

        def a_side(ref, r0, half):
            h0 = r0 + half
            if not isinstance(r0, int):
                h0 = pl.multiple_of(h0, half)
            a11 = ref[pl.ds(r0, half), pl.ds(0, HK)]
            a12 = ref[pl.ds(r0, half), pl.ds(HK, HK)]
            a21 = ref[pl.ds(h0, half), pl.ds(0, HK)]
            a22 = ref[pl.ds(h0, half), pl.ds(HK, HK)]
            L = _left_operands(*[v.astype(F32) for v in (a11, a12, a21, a22)])
            L = [v.astype(BF16) for v in L]
            L[2], L[3] = a11, a22
            return L

        def square_sums(src, dst):
            st = HK // sqparts

            def body(k, _):
                r = pl.multiple_of(k * st, st)
                blocks = [src[pl.ds(pl.multiple_of(kk + r, st), st), pl.ds(o, HK)].astype(F32)
                          for kk in (0, HK) for o in (0, HK)]
                for j, v in enumerate(_right_sums(*blocks)):
                    dst[j, pl.ds(r, st), :] = v.astype(BF16)
                return 0
            lax.fori_loop(0, sqparts, body, 0)

        def ffn_sums(k, _):
            c, part = k // nsub, k % nsub
            oa = pl.multiple_of(c * NC, NC)
            ob = pl.multiple_of(HF + c * NC, NC)
            for src, dst in ((w1_v, r1_v), (w3_v, r3_v), (w2_v, r2_v)):
                st = dst.shape[2] // nsub
                r = pl.multiple_of(part * st, st)
                if src is w2_v:
                    blocks = [src[pl.ds(pl.multiple_of(o + r, st), st), pl.ds(kk, HK)] for o in (oa, ob) for kk in (0, HK)]
                else:
                    blocks = [src[pl.ds(pl.multiple_of(kk + r, st), st), pl.ds(o, NC)] for kk in (0, HK) for o in (oa, ob)]
                for j, v in enumerate(_right_sums(*[b.astype(F32) for b in blocks])):
                    dst[c, j, pl.ds(r, st), :] = v.astype(BF16)
            return 0

        def ffn_products(L, w_ref, r_ref, c):
            if w_ref is w2_v:
                b11 = w_ref[pl.ds(c * NC, NC), pl.ds(0, HK)]
                b22 = w_ref[pl.ds(HF + c * NC, NC), pl.ds(HK, HK)]
            else:
                b11 = w_ref[pl.ds(0, HK), pl.ds(c * NC, NC)]
                b22 = w_ref[pl.ds(HK, HK), pl.ds(HF + c * NC, NC)]
            return _products(L, [r_ref[c, j] for j in range(5)], b11, b22)

        def proj(p, m):
            r0 = pl.multiple_of(m * T0, T0)
            h0 = pl.multiple_of(r0 + HT, HT)
            w, rq = wqkv_v.at[p], rq_v.at[p]
            M = _products(a_side(xn_v, r0, HT), [rq[j] for j in range(5)],
                          w[pl.ds(0, HK), pl.ds(0, HK)], w[pl.ds(HK, HK), pl.ds(HK, HK)])
            c11, c12, c21, c22 = _combine(M)
            qkv_v[p, pl.ds(r0, HT), pl.ds(0, HK)] = c11.astype(BF16)
            qkv_v[p, pl.ds(r0, HT), pl.ds(HK, HK)] = c12.astype(BF16)
            qkv_v[p, pl.ds(h0, HT), pl.ds(0, HK)] = c21.astype(BF16)
            qkv_v[p, pl.ds(h0, HT), pl.ds(HK, HK)] = c22.astype(BF16)

        z = jnp.zeros((HALO, 128), F32)
        if xsplit:
            xa, xb = x_rows(0, HT, 0), x_rows(HT, HT, nM)
            qkv_copy(0).start()
            xa.start()
            xb.start()
            x_copy(1).start()
            for e in range(8):
                k_scr[e, pl.ds(0, HALO), :] = z
                v_scr[e, pl.ds(0, HALO), :] = z
            with sc('a_wq'):
                qkv_copy(0).wait()
                square_sums(wqkv_v.at[0], rq_v.at[0])
            with sc('b_ln0'):
                xa.wait()
                ln_rows(0, 0, HT)
                xb.wait()
                for m in range(2, nM):
                    x_copy(m).start()
                ln_rows(HT, HT, HT)
        else:
            x_copy(0).start()
            qkv_copy(0).start()
            x_copy(1).start()
            for e in range(8):
                k_scr[e, pl.ds(0, HALO), :] = z
                v_scr[e, pl.ds(0, HALO), :] = z
            with sc('a_wait_x0'):
                x_copy(0).wait()
            with sc('b_ln0'):
                ln_rows(0, 0, T0)
            with sc('c_wq'):
                qkv_copy(0).wait()
                for m in range(2, nM):
                    x_copy(m).start()
                square_sums(wqkv_v.at[0], rq_v.at[0])

        def q_body(m, _):
            acts = {0: [qkv_copy(1).start, qkv_copy(2).start], nM - 2: [late[0].start], nM - 1: [late[1].start]}
            for k in range(nM - 1):
                acts.setdefault(k, []).append(x_copy(k + 1).wait)
            when_step(m, acts)
            proj(0, m)
            ln_rows(pl.multiple_of(jnp.minimum(m + 1, nM - 1) * T0, T0), pl.multiple_of((m + 1) * T0, T0), T0)
            return 0
        with sc('d_q'):
            lax.fori_loop(0, nM, q_body, 0)

        def kv_body(i, _):
            p = 1 + i // nM
            acts = {0: [qkv_copy(1).wait, qkv_copy(2).wait]}
            for k in range(2, len(late)):
                acts.setdefault(k - 2, []).append(late[k].start)
            when_step(i, acts)

            @pl.when(i % nM == 0)
            def _():
                square_sums(wqkv_v.at[p], rq_v.at[p])
            proj(p, i % nM)
            return 0
        with sc('e_kv'):
            lax.fori_loop(0, 2 * nM, kv_body, 0)

        with sc('f_sums'):
            for cp in late:
                cp.wait()
            lax.fori_loop(0, nC * nsub, ffn_sums, 0)

        laneR = lax.broadcasted_iota(jnp.int32, (R, 128), 1)
        m1 = (laneR & 1) == 0
        m2 = (laneR & 2) == 0
        laneH = lax.broadcasted_iota(jnp.int32, (R // 2, 128), 1)
        masksH = [(laneH & (4 << b)) == 0 for b in range(3)]
        rowR = lax.broadcasted_iota(jnp.int32, (R, 128), 0)
        laneP = lax.broadcasted_iota(jnp.int32, (T // 2, 128), 1)
        masksP = [(laneP & (4 << b)) == 0 for b in range(3)]
        scale = DH ** -0.5

        def tile_body(t, _):
            t0 = pl.multiple_of(t * T, T)
            slot = t % 2

            @pl.when(t >= 2)
            def _():
                out_copy(t - 2, slot).wait()

            for part, (dst, off) in enumerate(((q_scr, 0), (k_scr, HALO), (v_scr, HALO))):
                raw = pltpu.bitcast(qkv_v[part, pl.ds(t0, T), :], U32)
                tiles = _perm3([raw[:, c * 128:(c + 1) * 128] for c in range(8)], masksP)
                for e in range(8):
                    dst[e, pl.ds(off, T), :] = pltpu.bitcast(tiles[e], BF16).astype(F32)

            for rb in range(nR):
                r0 = rb * R
                q = [q_scr[e, pl.ds(r0, R), :] for e in range(8)]
                ls = []
                for j in range(W):
                    a = None
                    for e in range(8):
                        pr = q[e] * k_scr[e, pl.ds(HALO + r0 - DIL * j, R), :]
                        a = pr if a is None else a + pr
                    a = a + jnp.where(m1, pltpu.roll(a, 127, 1), pltpu.roll(a, 1, 1))
                    a = a + jnp.where(m2, pltpu.roll(a, 126, 1), pltpu.roll(a, 2, 1))
                    if r0 < DIL * j:
                        a = jnp.where(t0 + r0 + rowR >= DIL * j, a, -1e9 / scale)
                    ls.append(a)
                mx = ls[0]
                for j in range(1, W):
                    mx = jnp.maximum(mx, ls[j])
                ps = [jnp.exp2((l - mx) * (LOG2E * scale)) for l in ls]
                zs = ps[0]
                for j in range(1, W):
                    zs = zs + ps[j]
                inv = 1.0 / zs
                outs = []
                for e in range(8):
                    a = None
                    for j in range(W):
                        pr = ps[j] * v_scr[e, pl.ds(HALO + r0 - DIL * j, R), :]
                        a = pr if a is None else a + pr
                    outs.append(pltpu.bitcast((a * inv).astype(BF16), U32))
                outs = _perm3(outs, masksH)
                for c in range(8):
                    o_scr[pl.ds(r0, R), pl.ds(c * 128, 128)] = pltpu.bitcast(outs[c], BF16)

            L = a_side(xn_v, t0, T // 2)
            acc = [None] * 7
            for c in range(nC):
                g = _combine(ffn_products(L, w1_v, r1_v, c))
                u = _combine(ffn_products(L, w3_v, r3_v, c))
                h = [_silu_mul(g[i], u[i]) for i in range(4)]
                Lh = [v.astype(BF16) for v in _left_operands(*h)]
                M = ffn_products(Lh, w2_v, r2_v, c)
                acc = [m if a is None else a + m for a, m in zip(acc, M)]
            s_out = _dot(o_scr[...], wo_v[...])
            c11, c12, c21, c22 = _combine(acc)
            ffn = jnp.concatenate([jnp.concatenate([c11, c12], axis=1), jnp.concatenate([c21, c22], axis=1)], axis=0)

            for e in range(8):
                k_scr[e, pl.ds(0, HALO), :] = k_scr[e, pl.ds(T, HALO), :]
                v_scr[e, pl.ds(0, HALO), :] = v_scr[e, pl.ds(T, HALO), :]

            out_v[slot] = (x_v[pl.ds(t0, T), :].astype(F32) + _silu_mul(ffn, s_out)).astype(BF16)
            out_copy(t, slot).start()
            return 0

        with sc('g_main'):
            lax.fori_loop(0, nT, tile_body, 0)
        with sc('h_tail'):
            out_copy(nT - 2, (nT - 2) % 2).wait()
            out_copy(nT - 1, (nT - 1) % 2).wait()

    def fn(A_x, A_wqkv, A_wo, B_x, B_w1, B_w3, B_w2):
        del B_x
        hbm = pl.BlockSpec(memory_space=pl.ANY)
        out = pl.pallas_call(
            kernel,
            in_specs=[hbm] * 6,
            out_specs=hbm,
            out_shape=jax.ShapeDtypeStruct((S, D), A_x.dtype),
            scratch_shapes=[
                pltpu.VMEM((S, D), BF16),
                pltpu.VMEM((3, D, D), BF16), pltpu.VMEM((D, D), BF16),
                pltpu.VMEM((D, F), BF16), pltpu.VMEM((D, F), BF16), pltpu.VMEM((F, D), BF16),
                pltpu.VMEM((nC, 5, HK, NC), BF16), pltpu.VMEM((nC, 5, HK, NC), BF16),
                pltpu.VMEM((nC, 5, NC, HK), BF16), pltpu.VMEM((3, 5, HK, HK), BF16),
                pltpu.VMEM((S + T0, D), BF16),
                pltpu.VMEM((3, S, D), BF16),
                pltpu.VMEM((8, T, 128), F32), pltpu.VMEM((8, HALO + T, 128), F32), pltpu.VMEM((8, HALO + T, 128), F32),
                pltpu.VMEM((T, D), BF16), pltpu.VMEM((2, T, D), BF16),
                pltpu.SemaphoreType.DMA((nM + 1,)), pltpu.SemaphoreType.DMA((10,)), pltpu.SemaphoreType.DMA((2,)),
            ],
            compiler_params=pltpu.CompilerParams(vmem_limit_bytes=120 * 1024 * 1024, flags=flags),
        )(A_x.reshape(S, D), A_wqkv, A_wo, B_w1, B_w3, B_w2)
        return out.reshape(1, S, D)
    return fn


_impl = make_kernel(flags={'XLA_TPU_EVENLY_DISTRIBUTE_CRITICAL_NODES': True})


@jax.jit
def pallas_recurrent_scan__sliding_local_dilated__glu_gated_swiglu__prompt_kernel(
    A_x: jax.Array,
    A_wqkv: jax.Array,
    A_wo: jax.Array,
    B_x: jax.Array,
    B_w1: jax.Array,
    B_w3: jax.Array,
    B_w2: jax.Array,
):
    return _impl(A_x, A_wqkv, A_wo, B_x, B_w1, B_w3, B_w2)
```

```python
import contextlib

import jax
import jax.numpy as jnp
from jax import lax
from jax.experimental import pallas as pl
from jax.experimental.pallas import tpu as pltpu

F32 = jnp.float32
BF16 = jnp.bfloat16
U32 = jnp.uint32
S, D, F = 2048, 1024, 3584
H, DH, W, DIL = 32, 32, 8, 2
LOG2E = 1.4426950408889634
HALO = 16
HK, HF = D // 2, F // 2


def _dot(a, b):
    return jnp.dot(a, b, preferred_element_type=F32)


def _perm3(tiles, masks):
    for b in range(3):
        r = 4 << b
        m = masks[b]
        new = list(tiles)
        for c in range(8):
            if c & (1 << b):
                continue
            A, B = tiles[c], tiles[c | (1 << b)]
            new[c] = jnp.where(m, A, pltpu.roll(B, r, 1))
            new[c | (1 << b)] = jnp.where(m, pltpu.roll(A, 128 - r, 1), B)
        tiles = new
    return tiles


def _silu_mul(g, u):
    hg = 0.5 * g
    return (hg + hg * jnp.tanh(hg)) * u


def _left_operands(a11, a12, a21, a22):
    return [a11 + a22, a21 + a22, a11, a22, a11 + a12, a21 - a11, a12 - a22]


def _right_sums(b11, b12, b21, b22):
    return [b11 + b22, b12 - b22, b21 - b11, b11 + b12, b21 + b22]


ORDER = {'proj': (0, 1, 2, 3, 4, 5, 6), 'gu': (0, 1, 2, 3, 4, 5, 6), 'w2': (0, 1, 2, 3, 4, 5, 6), 'wo': (0, 1, 2, 3, 4, 5, 6)}


def _products(L, sums, b11, b22, order=(0, 1, 2, 3, 4, 5, 6)):
    R = [sums[0], b11, sums[1], sums[2], b22, sums[3], sums[4]]
    M = [None] * 7
    for i in order:
        M[i] = _dot(L[i], R[i])
    return M


def _combine(M):
    return (M[0] + M[3] - M[4] + M[6], M[2] + M[4], M[1] + M[3], M[0] - M[1] + M[2] + M[5])


def make_kernel(scopes=False, flags=None, T=256, T0=512, NC=256, R=32, nsub=16, sqparts=16, xsplit=False, order=None, qdirect=False, attn_after=False, norm_p=False, halo_top=True, wo_str=True, wo_pos=7):
    nT, nM, nC, nR = S // T, S // T0, HF // NC, T // R
    od = dict(ORDER)
    od.update(order or {})
    sc = (lambda n: jax.named_scope(n)) if scopes else (lambda n: contextlib.nullcontext())

    def kernel(x_hbm, wqkv_hbm, wo_hbm, w1_hbm, w3_hbm, w2_hbm, o_hbm,
               x_v, wqkv_v, wo_v, w1_v, w3_v, w2_v, r1_v, r3_v, r2_v, rq_v, ro_v, xn_v, qkv_v,
               q_scr, k_scr, v_scr, o_scr, out_v, xsem, wsem, osem):

        HT = T0 // 2

        def x_rows(r0, n, k):
            return pltpu.make_async_copy(x_hbm.at[pl.ds(r0, n), :], x_v.at[pl.ds(r0, n), :], xsem.at[k])

        def x_copy(m):
            return x_rows(m * T0, T0, m)

        def qkv_copy(p):
            return pltpu.make_async_copy(wqkv_hbm.at[:, pl.ds(p * D, D)], wqkv_v.at[p], wsem.at[p])

        def cols_copy(src, dst, c, k):
            return pltpu.make_async_copy(src.at[:, pl.ds(c * HF, HF)], dst.at[:, pl.ds(c * HF, HF)], wsem.at[k])

        def rows_copy(src, dst, c, k):
            return pltpu.make_async_copy(src.at[pl.ds(c * HF, HF), :], dst.at[pl.ds(c * HF, HF), :], wsem.at[k])

        late = [cols_copy(w1_hbm, w1_v, 0, 3), cols_copy(w1_hbm, w1_v, 1, 4),
                cols_copy(w3_hbm, w3_v, 0, 5), cols_copy(w3_hbm, w3_v, 1, 6),
                rows_copy(w2_hbm, w2_v, 0, 7), rows_copy(w2_hbm, w2_v, 1, 8),
                pltpu.make_async_copy(wo_hbm, wo_v, wsem.at[9])]

        def out_copy(t, slot):
            return pltpu.make_async_copy(out_v.at[slot], o_hbm.at[pl.ds(t * T, T), :], osem.at[slot])

        def when_step(i, acts):
            for k, fs in sorted(acts.items()):
                @pl.when(i == k)
                def _(fs=fs):
                    for f in fs:
                        f()

        def ln_rows(src0, dst0, n):
            x = x_v[pl.ds(src0, n), :].astype(F32)
            mu = jnp.mean(x, axis=-1, keepdims=True)
            xc = x - mu
            var = jnp.mean(xc * xc, axis=-1, keepdims=True)
            xn_v[pl.ds(dst0, n), :] = (xc / jnp.sqrt(var + 1e-5)).astype(BF16)

        def a_side(ref, r0, half):
            h0 = r0 + half
            if not isinstance(r0, int):
                h0 = pl.multiple_of(h0, half)
            a11 = ref[pl.ds(r0, half), pl.ds(0, HK)]
            a12 = ref[pl.ds(r0, half), pl.ds(HK, HK)]
            a21 = ref[pl.ds(h0, half), pl.ds(0, HK)]
            a22 = ref[pl.ds(h0, half), pl.ds(HK, HK)]
            L = _left_operands(*[v.astype(F32) for v in (a11, a12, a21, a22)])
            L = [v.astype(BF16) for v in L]
            L[2], L[3] = a11, a22
            return L

        def square_sums(src, dst):
            st = HK // sqparts

            def body(k, _):
                r = pl.multiple_of(k * st, st)
                blocks = [src[pl.ds(pl.multiple_of(kk + r, st), st), pl.ds(o, HK)].astype(F32)
                          for kk in (0, HK) for o in (0, HK)]
                for j, v in enumerate(_right_sums(*blocks)):
                    dst[j, pl.ds(r, st), :] = v.astype(BF16)
                return 0
            lax.fori_loop(0, sqparts, body, 0)

        def ffn_sums(k, _):
            c, part = k // nsub, k % nsub
            oa = pl.multiple_of(c * NC, NC)
            ob = pl.multiple_of(HF + c * NC, NC)
            for src, dst in ((w1_v, r1_v), (w3_v, r3_v), (w2_v, r2_v)):
                st = dst.shape[2] // nsub
                r = pl.multiple_of(part * st, st)
                if src is w2_v:
                    blocks = [src[pl.ds(pl.multiple_of(o + r, st), st), pl.ds(kk, HK)] for o in (oa, ob) for kk in (0, HK)]
                else:
                    blocks = [src[pl.ds(pl.multiple_of(kk + r, st), st), pl.ds(o, NC)] for kk in (0, HK) for o in (oa, ob)]
                for j, v in enumerate(_right_sums(*[b.astype(F32) for b in blocks])):
                    dst[c, j, pl.ds(r, st), :] = v.astype(BF16)
            return 0

        def ffn_products(L, w_ref, r_ref, c):
            if w_ref is w2_v:
                b11 = w_ref[pl.ds(c * NC, NC), pl.ds(0, HK)]
                b22 = w_ref[pl.ds(HF + c * NC, NC), pl.ds(HK, HK)]
            else:
                b11 = w_ref[pl.ds(0, HK), pl.ds(c * NC, NC)]
                b22 = w_ref[pl.ds(HK, HK), pl.ds(HF + c * NC, NC)]
            return _products(L, [r_ref[c, j] for j in range(5)], b11, b22, od['w2' if w_ref is w2_v else 'gu'])

        def proj(p, m):
            r0 = pl.multiple_of(m * T0, T0)
            h0 = pl.multiple_of(r0 + HT, HT)
            w, rq = wqkv_v.at[p], rq_v.at[p]
            M = _products(a_side(xn_v, r0, HT), [rq[j] for j in range(5)],
                          w[pl.ds(0, HK), pl.ds(0, HK)], w[pl.ds(HK, HK), pl.ds(HK, HK)], od['proj'])
            c11, c12, c21, c22 = _combine(M)
            qkv_v[p, pl.ds(r0, HT), pl.ds(0, HK)] = c11.astype(BF16)
            qkv_v[p, pl.ds(r0, HT), pl.ds(HK, HK)] = c12.astype(BF16)
            qkv_v[p, pl.ds(h0, HT), pl.ds(0, HK)] = c21.astype(BF16)
            qkv_v[p, pl.ds(h0, HT), pl.ds(HK, HK)] = c22.astype(BF16)

        z = jnp.zeros((HALO, 128), F32)
        if xsplit:
            xa, xb = x_rows(0, HT, 0), x_rows(HT, HT, nM)
            qkv_copy(0).start()
            xa.start()
            xb.start()
            x_copy(1).start()
            for e in range(8):
                k_scr[e, pl.ds(T if halo_top else 0, HALO), :] = z
                v_scr[e, pl.ds(T if halo_top else 0, HALO), :] = z
            with sc('a_wq'):
                qkv_copy(0).wait()
                square_sums(wqkv_v.at[0], rq_v.at[0])
            with sc('b_ln0'):
                xa.wait()
                ln_rows(0, 0, HT)
                xb.wait()
                for m in range(2, nM):
                    x_copy(m).start()
                ln_rows(HT, HT, HT)
        else:
            x_copy(0).start()
            qkv_copy(0).start()
            x_copy(1).start()
            for e in range(8):
                k_scr[e, pl.ds(T if halo_top else 0, HALO), :] = z
                v_scr[e, pl.ds(T if halo_top else 0, HALO), :] = z
            with sc('a_wait_x0'):
                x_copy(0).wait()
            with sc('b_ln0'):
                ln_rows(0, 0, T0)
            with sc('c_wq'):
                qkv_copy(0).wait()
                for m in range(2, nM):
                    x_copy(m).start()
                square_sums(wqkv_v.at[0], rq_v.at[0])

        def q_body(m, _):
            acts = {0: [qkv_copy(1).start, qkv_copy(2).start], nM - 2: [late[0].start], nM - 1: [late[1].start]}
            for k in range(nM - 1):
                acts.setdefault(k, []).append(x_copy(k + 1).wait)
            when_step(m, acts)
            proj(0, m)
            ln_rows(pl.multiple_of(jnp.minimum(m + 1, nM - 1) * T0, T0), pl.multiple_of((m + 1) * T0, T0), T0)
            return 0
        with sc('d_q'):
            lax.fori_loop(0, nM, q_body, 0)

        def kv_body(i, _):
            p = 1 + i // nM
            acts = {0: [qkv_copy(1).wait, qkv_copy(2).wait]}
            for k in range(2, len(late)):
                acts.setdefault(k - 2, []).append(late[k].start)
            when_step(i, acts)

            @pl.when(i % nM == 0)
            def _():
                square_sums(wqkv_v.at[p], rq_v.at[p])
            proj(p, i % nM)
            return 0
        with sc('e_kv'):
            lax.fori_loop(0, 2 * nM, kv_body, 0)

        with sc('f_sums'):
            for cp in late:
                cp.wait()
            lax.fori_loop(0, nC * nsub, ffn_sums, 0)
            if wo_str:
                square_sums(wo_v, ro_v)

        laneR = lax.broadcasted_iota(jnp.int32, (R, 128), 1)
        m1 = (laneR & 1) == 0
        m2 = (laneR & 2) == 0
        laneH = lax.broadcasted_iota(jnp.int32, (R // 2, 128), 1)
        masksH = [(laneH & (4 << b)) == 0 for b in range(3)]
        rowR = lax.broadcasted_iota(jnp.int32, (R, 128), 0)
        laneP = lax.broadcasted_iota(jnp.int32, (T // 2, 128), 1)
        masksP = [(laneP & (4 << b)) == 0 for b in range(3)]
        scale = DH ** -0.5

        def tile_body(t, _):
            t0 = pl.multiple_of(t * T, T)
            slot = t % 2

            @pl.when(t >= 2)
            def _():
                out_copy(t - 2, slot).wait()

            def halo():
                for e in range(8):
                    k_scr[e, pl.ds(0, HALO), :] = k_scr[e, pl.ds(T, HALO), :]
                    v_scr[e, pl.ds(0, HALO), :] = v_scr[e, pl.ds(T, HALO), :]
            if halo_top:
                halo()

            for part, (dst, off) in enumerate(((q_scr, 0), (k_scr, HALO), (v_scr, HALO))):
                raw = pltpu.bitcast(qkv_v[part, pl.ds(t0, T), :], U32)
                tiles = _perm3([raw[:, c * 128:(c + 1) * 128] for c in range(8)], masksP)
                if part == 0 and qdirect:
                    qfull = [pltpu.bitcast(tiles[e], BF16).astype(F32) for e in range(8)]
                    continue
                for e in range(8):
                    dst[e, pl.ds(off, T), :] = pltpu.bitcast(tiles[e], BF16).astype(F32)

            for rb in range(nR):
                r0 = rb * R
                q = [qfull[e][r0:r0 + R] for e in range(8)] if qdirect else [q_scr[e, pl.ds(r0, R), :] for e in range(8)]
                ls = []
                for j in range(W):
                    a = None
                    for e in range(8):
                        pr = q[e] * k_scr[e, pl.ds(HALO + r0 - DIL * j, R), :]
                        a = pr if a is None else a + pr
                    a = a + jnp.where(m1, pltpu.roll(a, 127, 1), pltpu.roll(a, 1, 1))
                    a = a + jnp.where(m2, pltpu.roll(a, 126, 1), pltpu.roll(a, 2, 1))
                    if r0 < DIL * j:
                        a = jnp.where(t0 + r0 + rowR >= DIL * j, a, -1e9 / scale)
                    ls.append(a)
                mx = ls[0]
                for j in range(1, W):
                    mx = jnp.maximum(mx, ls[j])
                ps = [jnp.exp2((l - mx) * (LOG2E * scale)) for l in ls]
                zs = ps[0]
                for j in range(1, W):
                    zs = zs + ps[j]
                inv = 1.0 / zs
                if norm_p:
                    ps = [p_ * inv for p_ in ps]
                outs = []
                for e in range(8):
                    a = None
                    for j in range(W):
                        pr = ps[j] * v_scr[e, pl.ds(HALO + r0 - DIL * j, R), :]
                        a = pr if a is None else a + pr
                    outs.append(pltpu.bitcast((a if norm_p else a * inv).astype(BF16), U32))
                outs = _perm3(outs, masksH)
                for c in range(8):
                    o_scr[pl.ds(r0, R), pl.ds(c * 128, 128)] = pltpu.bitcast(outs[c], BF16)

            L = a_side(xn_v, t0, T // 2)
            acc = [None] * 7
            def wo_proj():
                if not wo_str:
                    return _dot(o_scr[...], wo_v[...])
                M = _products(a_side(o_scr, 0, T // 2), [ro_v[j] for j in range(5)],
                              wo_v[pl.ds(0, HK), pl.ds(0, HK)], wo_v[pl.ds(HK, HK), pl.ds(HK, HK)], od['wo'])
                s11, s12, s21, s22 = _combine(M)
                return jnp.concatenate([jnp.concatenate([s11, s12], axis=1), jnp.concatenate([s21, s22], axis=1)], axis=0)

            for c in range(nC):
                if c == wo_pos:
                    s_out = wo_proj()
                g = _combine(ffn_products(L, w1_v, r1_v, c))
                u = _combine(ffn_products(L, w3_v, r3_v, c))
                h = [_silu_mul(g[i], u[i]) for i in range(4)]
                Lh = [v.astype(BF16) for v in _left_operands(*h)]
                M = ffn_products(Lh, w2_v, r2_v, c)
                acc = [m if a is None else a + m for a, m in zip(acc, M)]
            if wo_pos >= nC:
                s_out = wo_proj()
            c11, c12, c21, c22 = _combine(acc)
            ffn = jnp.concatenate([jnp.concatenate([c11, c12], axis=1), jnp.concatenate([c21, c22], axis=1)], axis=0)

            if not halo_top:
                halo()
            out_v[slot] = (x_v[pl.ds(t0, T), :].astype(F32) + _silu_mul(ffn, s_out)).astype(BF16)
            out_copy(t, slot).start()
            return 0

        with sc('g_main'):
            lax.fori_loop(0, nT, tile_body, 0)
        with sc('h_tail'):
            out_copy(nT - 2, (nT - 2) % 2).wait()
            out_copy(nT - 1, (nT - 1) % 2).wait()

    def fn(A_x, A_wqkv, A_wo, B_x, B_w1, B_w3, B_w2):
        del B_x
        hbm = pl.BlockSpec(memory_space=pl.ANY)
        out = pl.pallas_call(
            kernel,
            in_specs=[hbm] * 6,
            out_specs=hbm,
            out_shape=jax.ShapeDtypeStruct((S, D), A_x.dtype),
            scratch_shapes=[
                pltpu.VMEM((S, D), BF16),
                pltpu.VMEM((3, D, D), BF16), pltpu.VMEM((D, D), BF16),
                pltpu.VMEM((D, F), BF16), pltpu.VMEM((D, F), BF16), pltpu.VMEM((F, D), BF16),
                pltpu.VMEM((nC, 5, HK, NC), BF16), pltpu.VMEM((nC, 5, HK, NC), BF16),
                pltpu.VMEM((nC, 5, NC, HK), BF16), pltpu.VMEM((3, 5, HK, HK), BF16), pltpu.VMEM((5, HK, HK), BF16),
                pltpu.VMEM((S + T0, D), BF16),
                pltpu.VMEM((3, S, D), BF16),
                pltpu.VMEM((8, T, 128), F32), pltpu.VMEM((8, HALO + T, 128), F32), pltpu.VMEM((8, HALO + T, 128), F32),
                pltpu.VMEM((T, D), BF16), pltpu.VMEM((2, T, D), BF16),
                pltpu.SemaphoreType.DMA((nM + 1,)), pltpu.SemaphoreType.DMA((10,)), pltpu.SemaphoreType.DMA((2,)),
            ],
            compiler_params=pltpu.CompilerParams(vmem_limit_bytes=120 * 1024 * 1024, flags=flags),
        )(A_x.reshape(S, D), A_wqkv, A_wo, B_w1, B_w3, B_w2)
        return out.reshape(1, S, D)
    return fn


_impl = make_kernel(flags={'XLA_TPU_EVENLY_DISTRIBUTE_CRITICAL_NODES': True}, wo_str=True, norm_p=True, R=16, order={'wo': (2, 0, 3, 1, 4, 5, 6), 'w2': (6, 5, 1, 2, 0, 3, 4), 'gu': (0, 1, 2, 5, 4, 3, 6), 'proj': (6, 0, 2, 5, 3, 4, 1)})


@jax.jit
def pallas_recurrent_scan__sliding_local_dilated__glu_gated_swiglu__prompt_kernel(
    A_x: jax.Array,
    A_wqkv: jax.Array,
    A_wo: jax.Array,
    B_x: jax.Array,
    B_w1: jax.Array,
    B_w3: jax.Array,
    B_w2: jax.Array,
):
    return _impl(A_x, A_wqkv, A_wo, B_x, B_w1, B_w3, B_w2)
```

```python
import contextlib

import jax
import jax.numpy as jnp
from jax import lax
from jax.experimental import pallas as pl
from jax.experimental.pallas import tpu as pltpu

F32 = jnp.float32
BF16 = jnp.bfloat16
U32 = jnp.uint32
S, D, F = 2048, 1024, 3584
H, DH, W, DIL = 32, 32, 8, 2
LOG2E = 1.4426950408889634
HALO = 16
HK, HF = D // 2, F // 2


def _dot(a, b):
    return jnp.dot(a, b, preferred_element_type=F32)


def _perm3(tiles, masks):
    for b in range(3):
        r = 4 << b
        m = masks[b]
        new = list(tiles)
        for c in range(8):
            if c & (1 << b):
                continue
            A, B = tiles[c], tiles[c | (1 << b)]
            new[c] = jnp.where(m, A, pltpu.roll(B, r, 1))
            new[c | (1 << b)] = jnp.where(m, pltpu.roll(A, 128 - r, 1), B)
        tiles = new
    return tiles


def _silu_mul(g, u):
    hg = 0.5 * g
    return (hg + hg * jnp.tanh(hg)) * u


def _left_operands(a11, a12, a21, a22):
    return [a11 + a22, a21 + a22, a11, a22, a11 + a12, a21 - a11, a12 - a22]


def _right_sums(b11, b12, b21, b22):
    return [b11 + b22, b12 - b22, b21 - b11, b11 + b12, b21 + b22]


ORDER_QKV = (6, 0, 5, 3, 2, 4, 1)
ORDER_UP = (0, 1, 2, 5, 4, 3, 6)
ORDER_DOWN = (6, 2, 1, 5, 0, 3, 4)
ORDER_OUT = (2, 0, 1, 4, 3, 5, 6)


def _products(L, sums, b11, b22, order):
    R = [sums[0], b11, sums[1], sums[2], b22, sums[3], sums[4]]
    M = [None] * 7
    for i in order:
        M[i] = _dot(L[i], R[i])
    return M


def _combine(M):
    return (M[0] + M[3] - M[4] + M[6], M[2] + M[4], M[1] + M[3], M[0] - M[1] + M[2] + M[5])


def make_kernel(scopes=False, flags=None, T=256, T0=512, NC=256, R=16, nsub=16, sqparts=16):
    nT, nM, nC, nR = S // T, S // T0, HF // NC, T // R
    sc = (lambda n: jax.named_scope(n)) if scopes else (lambda n: contextlib.nullcontext())

    def kernel(x_hbm, wqkv_hbm, wo_hbm, w1_hbm, w3_hbm, w2_hbm, o_hbm,
               x_v, wqkv_v, wo_v, w1_v, w3_v, w2_v, r1_v, r3_v, r2_v, rq_v, ro_v, xn_v, qkv_v,
               q_scr, k_scr, v_scr, o_scr, out_v, xsem, wsem, osem):

        HT = T0 // 2

        def x_copy(m):
            return pltpu.make_async_copy(x_hbm.at[pl.ds(m * T0, T0), :], x_v.at[pl.ds(m * T0, T0), :], xsem.at[m])

        def qkv_copy(p):
            return pltpu.make_async_copy(wqkv_hbm.at[:, pl.ds(p * D, D)], wqkv_v.at[p], wsem.at[p])

        def cols_copy(src, dst, c, k):
            return pltpu.make_async_copy(src.at[:, pl.ds(c * HF, HF)], dst.at[:, pl.ds(c * HF, HF)], wsem.at[k])

        def rows_copy(src, dst, c, k):
            return pltpu.make_async_copy(src.at[pl.ds(c * HF, HF), :], dst.at[pl.ds(c * HF, HF), :], wsem.at[k])

        late = [cols_copy(w1_hbm, w1_v, 0, 3), cols_copy(w1_hbm, w1_v, 1, 4),
                cols_copy(w3_hbm, w3_v, 0, 5), cols_copy(w3_hbm, w3_v, 1, 6),
                rows_copy(w2_hbm, w2_v, 0, 7), rows_copy(w2_hbm, w2_v, 1, 8),
                pltpu.make_async_copy(wo_hbm, wo_v, wsem.at[9])]

        def out_copy(t, slot):
            return pltpu.make_async_copy(out_v.at[slot], o_hbm.at[pl.ds(t * T, T), :], osem.at[slot])

        def when_step(i, acts):
            for k, fs in sorted(acts.items()):
                @pl.when(i == k)
                def _(fs=fs):
                    for f in fs:
                        f()

        def ln_rows(src0, dst0, n):
            x = x_v[pl.ds(src0, n), :].astype(F32)
            mu = jnp.mean(x, axis=-1, keepdims=True)
            xc = x - mu
            var = jnp.mean(xc * xc, axis=-1, keepdims=True)
            xn_v[pl.ds(dst0, n), :] = (xc / jnp.sqrt(var + 1e-5)).astype(BF16)

        def a_side(ref, r0, half):
            h0 = r0 + half
            if not isinstance(r0, int):
                h0 = pl.multiple_of(h0, half)
            a11 = ref[pl.ds(r0, half), pl.ds(0, HK)]
            a12 = ref[pl.ds(r0, half), pl.ds(HK, HK)]
            a21 = ref[pl.ds(h0, half), pl.ds(0, HK)]
            a22 = ref[pl.ds(h0, half), pl.ds(HK, HK)]
            L = _left_operands(*[v.astype(F32) for v in (a11, a12, a21, a22)])
            L = [v.astype(BF16) for v in L]
            L[2], L[3] = a11, a22
            return L

        def square_sums(src, dst):
            st = HK // sqparts

            def body(k, _):
                r = pl.multiple_of(k * st, st)
                blocks = [src[pl.ds(pl.multiple_of(kk + r, st), st), pl.ds(o, HK)].astype(F32)
                          for kk in (0, HK) for o in (0, HK)]
                for j, v in enumerate(_right_sums(*blocks)):
                    dst[j, pl.ds(r, st), :] = v.astype(BF16)
                return 0
            lax.fori_loop(0, sqparts, body, 0)

        def ffn_sums(k, _):
            c, part = k // nsub, k % nsub
            oa = pl.multiple_of(c * NC, NC)
            ob = pl.multiple_of(HF + c * NC, NC)
            for src, dst in ((w1_v, r1_v), (w3_v, r3_v), (w2_v, r2_v)):
                st = dst.shape[2] // nsub
                r = pl.multiple_of(part * st, st)
                if src is w2_v:
                    blocks = [src[pl.ds(pl.multiple_of(o + r, st), st), pl.ds(kk, HK)] for o in (oa, ob) for kk in (0, HK)]
                else:
                    blocks = [src[pl.ds(pl.multiple_of(kk + r, st), st), pl.ds(o, NC)] for kk in (0, HK) for o in (oa, ob)]
                for j, v in enumerate(_right_sums(*[b.astype(F32) for b in blocks])):
                    dst[c, j, pl.ds(r, st), :] = v.astype(BF16)
            return 0

        def ffn_products(L, w_ref, r_ref, c, order):
            if w_ref is w2_v:
                b11 = w_ref[pl.ds(c * NC, NC), pl.ds(0, HK)]
                b22 = w_ref[pl.ds(HF + c * NC, NC), pl.ds(HK, HK)]
            else:
                b11 = w_ref[pl.ds(0, HK), pl.ds(c * NC, NC)]
                b22 = w_ref[pl.ds(HK, HK), pl.ds(HF + c * NC, NC)]
            return _products(L, [r_ref[c, j] for j in range(5)], b11, b22, order)

        def proj(p, m):
            r0 = pl.multiple_of(m * T0, T0)
            h0 = pl.multiple_of(r0 + HT, HT)
            w, rq = wqkv_v.at[p], rq_v.at[p]
            M = _products(a_side(xn_v, r0, HT), [rq[j] for j in range(5)],
                          w[pl.ds(0, HK), pl.ds(0, HK)], w[pl.ds(HK, HK), pl.ds(HK, HK)], ORDER_QKV)
            c11, c12, c21, c22 = _combine(M)
            qkv_v[p, pl.ds(r0, HT), pl.ds(0, HK)] = c11.astype(BF16)
            qkv_v[p, pl.ds(r0, HT), pl.ds(HK, HK)] = c12.astype(BF16)
            qkv_v[p, pl.ds(h0, HT), pl.ds(0, HK)] = c21.astype(BF16)
            qkv_v[p, pl.ds(h0, HT), pl.ds(HK, HK)] = c22.astype(BF16)

        z = jnp.zeros((HALO, 128), F32)
        x_copy(0).start()
        qkv_copy(0).start()
        x_copy(1).start()
        for e in range(8):
            k_scr[e, pl.ds(T, HALO), :] = z
            v_scr[e, pl.ds(T, HALO), :] = z
        with sc('a_wait_x0'):
            x_copy(0).wait()
        with sc('b_ln0'):
            ln_rows(0, 0, T0)
        with sc('c_wq'):
            qkv_copy(0).wait()
            for m in range(2, nM):
                x_copy(m).start()
            square_sums(wqkv_v.at[0], rq_v.at[0])

        def q_body(m, _):
            acts = {0: [qkv_copy(1).start, qkv_copy(2).start], nM - 2: [late[0].start], nM - 1: [late[1].start]}
            for k in range(nM - 1):
                acts.setdefault(k, []).append(x_copy(k + 1).wait)
            when_step(m, acts)
            proj(0, m)
            ln_rows(pl.multiple_of(jnp.minimum(m + 1, nM - 1) * T0, T0), pl.multiple_of((m + 1) * T0, T0), T0)
            return 0
        with sc('d_q'):
            lax.fori_loop(0, nM, q_body, 0)

        def kv_body(i, _):
            p = 1 + i // nM
            acts = {0: [qkv_copy(1).wait, qkv_copy(2).wait]}
            for k in range(2, len(late)):
                acts.setdefault(k - 2, []).append(late[k].start)
            when_step(i, acts)

            @pl.when(i % nM == 0)
            def _():
                square_sums(wqkv_v.at[p], rq_v.at[p])
            proj(p, i % nM)
            return 0
        with sc('e_kv'):
            lax.fori_loop(0, 2 * nM, kv_body, 0)

        with sc('f_sums'):
            for cp in late:
                cp.wait()
            lax.fori_loop(0, nC * nsub, ffn_sums, 0)
            square_sums(wo_v, ro_v)

        laneR = lax.broadcasted_iota(jnp.int32, (R, 128), 1)
        m1 = (laneR & 1) == 0
        m2 = (laneR & 2) == 0
        laneH = lax.broadcasted_iota(jnp.int32, (R // 2, 128), 1)
        masksH = [(laneH & (4 << b)) == 0 for b in range(3)]
        rowR = lax.broadcasted_iota(jnp.int32, (R, 128), 0)
        laneP = lax.broadcasted_iota(jnp.int32, (T // 2, 128), 1)
        masksP = [(laneP & (4 << b)) == 0 for b in range(3)]
        scale = DH ** -0.5

        def tile_body(t, _):
            t0 = pl.multiple_of(t * T, T)
            slot = t % 2

            @pl.when(t >= 2)
            def _():
                out_copy(t - 2, slot).wait()

            for e in range(8):
                k_scr[e, pl.ds(0, HALO), :] = k_scr[e, pl.ds(T, HALO), :]
                v_scr[e, pl.ds(0, HALO), :] = v_scr[e, pl.ds(T, HALO), :]

            for part, (dst, off) in enumerate(((q_scr, 0), (k_scr, HALO), (v_scr, HALO))):
                raw = pltpu.bitcast(qkv_v[part, pl.ds(t0, T), :], U32)
                tiles = _perm3([raw[:, c * 128:(c + 1) * 128] for c in range(8)], masksP)
                for e in range(8):
                    dst[e, pl.ds(off, T), :] = pltpu.bitcast(tiles[e], BF16).astype(F32)

            for rb in range(nR):
                r0 = rb * R
                q = [q_scr[e, pl.ds(r0, R), :] for e in range(8)]
                ls = []
                for j in range(W):
                    a = None
                    for e in range(8):
                        pr = q[e] * k_scr[e, pl.ds(HALO + r0 - DIL * j, R), :]
                        a = pr if a is None else a + pr
                    a = a + jnp.where(m1, pltpu.roll(a, 127, 1), pltpu.roll(a, 1, 1))
                    a = a + jnp.where(m2, pltpu.roll(a, 126, 1), pltpu.roll(a, 2, 1))
                    if r0 < DIL * j:
                        a = jnp.where(t0 + r0 + rowR >= DIL * j, a, -1e9 / scale)
                    ls.append(a)
                mx = ls[0]
                for j in range(1, W):
                    mx = jnp.maximum(mx, ls[j])
                ps = [jnp.exp2((l - mx) * (LOG2E * scale)) for l in ls]
                zs = ps[0]
                for j in range(1, W):
                    zs = zs + ps[j]
                inv = 1.0 / zs
                ps = [p_ * inv for p_ in ps]
                outs = []
                for e in range(8):
                    a = None
                    for j in range(W):
                        pr = ps[j] * v_scr[e, pl.ds(HALO + r0 - DIL * j, R), :]
                        a = pr if a is None else a + pr
                    outs.append(pltpu.bitcast(a.astype(BF16), U32))
                outs = _perm3(outs, masksH)
                for c in range(8):
                    o_scr[pl.ds(r0, R), pl.ds(c * 128, 128)] = pltpu.bitcast(outs[c], BF16)

            L = a_side(xn_v, t0, T // 2)
            acc = [None] * 7
            for c in range(nC):
                Mg, Mu = [None] * 7, [None] * 7
                for i in ORDER_UP:
                    Mg[i] = ffn_products(L, w1_v, r1_v, c, (i,))[i]
                    Mu[i] = ffn_products(L, w3_v, r3_v, c, (i,))[i]
                g, u = _combine(Mg), _combine(Mu)
                h = [_silu_mul(g[i], u[i]) for i in range(4)]
                Lh = [v.astype(BF16) for v in _left_operands(*h)]
                M = ffn_products(Lh, w2_v, r2_v, c, ORDER_DOWN)
                acc = [m if a is None else a + m for a, m in zip(acc, M)]
            s11, s12, s21, s22 = _combine(_products(
                a_side(o_scr, 0, T // 2), [ro_v[j] for j in range(5)],
                wo_v[pl.ds(0, HK), pl.ds(0, HK)], wo_v[pl.ds(HK, HK), pl.ds(HK, HK)], ORDER_OUT))
            s_out = jnp.concatenate([jnp.concatenate([s11, s12], axis=1), jnp.concatenate([s21, s22], axis=1)], axis=0)
            c11, c12, c21, c22 = _combine(acc)
            ffn = jnp.concatenate([jnp.concatenate([c11, c12], axis=1), jnp.concatenate([c21, c22], axis=1)], axis=0)

            out_v[slot] = (x_v[pl.ds(t0, T), :].astype(F32) + _silu_mul(ffn, s_out)).astype(BF16)
            out_copy(t, slot).start()
            return 0

        with sc('g_main'):
            lax.fori_loop(0, nT, tile_body, 0)
        with sc('h_tail'):
            out_copy(nT - 2, (nT - 2) % 2).wait()
            out_copy(nT - 1, (nT - 1) % 2).wait()

    def fn(A_x, A_wqkv, A_wo, B_x, B_w1, B_w3, B_w2):
        del B_x
        hbm = pl.BlockSpec(memory_space=pl.ANY)
        out = pl.pallas_call(
            kernel,
            in_specs=[hbm] * 6,
            out_specs=hbm,
            out_shape=jax.ShapeDtypeStruct((S, D), A_x.dtype),
            scratch_shapes=[
                pltpu.VMEM((S, D), BF16),
                pltpu.VMEM((3, D, D), BF16), pltpu.VMEM((D, D), BF16),
                pltpu.VMEM((D, F), BF16), pltpu.VMEM((D, F), BF16), pltpu.VMEM((F, D), BF16),
                pltpu.VMEM((nC, 5, HK, NC), BF16), pltpu.VMEM((nC, 5, HK, NC), BF16),
                pltpu.VMEM((nC, 5, NC, HK), BF16), pltpu.VMEM((3, 5, HK, HK), BF16), pltpu.VMEM((5, HK, HK), BF16),
                pltpu.VMEM((S + T0, D), BF16),
                pltpu.VMEM((3, S, D), BF16),
                pltpu.VMEM((8, T, 128), F32), pltpu.VMEM((8, HALO + T, 128), F32), pltpu.VMEM((8, HALO + T, 128), F32),
                pltpu.VMEM((T, D), BF16), pltpu.VMEM((2, T, D), BF16),
                pltpu.SemaphoreType.DMA((nM,)), pltpu.SemaphoreType.DMA((10,)), pltpu.SemaphoreType.DMA((2,)),
            ],
            compiler_params=pltpu.CompilerParams(vmem_limit_bytes=120 * 1024 * 1024, flags=flags),
        )(A_x.reshape(S, D), A_wqkv, A_wo, B_w1, B_w3, B_w2)
        return out.reshape(1, S, D)
    return fn


_impl = make_kernel(flags={'XLA_TPU_EVENLY_DISTRIBUTE_CRITICAL_NODES': True})


@jax.jit
def pallas_recurrent_scan__sliding_local_dilated__glu_gated_swiglu__prompt_kernel(
    A_x: jax.Array,
    A_wqkv: jax.Array,
    A_wo: jax.Array,
    B_x: jax.Array,
    B_w1: jax.Array,
    B_w3: jax.Array,
    B_w2: jax.Array,
):
    return _impl(A_x, A_wqkv, A_wo, B_x, B_w1, B_w3, B_w2)
```
